```python
import jax
import jax.numpy as jnp

def _softmax(x, axis=-1):
    return jax.nn.softmax(x, axis=axis)
def _gelu(x):
    return jax.nn.gelu(x, approximate=True)
def _silu(x):
    return jax.nn.silu(x)
def _sigmoid(x):
    return jax.nn.sigmoid(x)
def _layernorm(x, axis=-1, eps=1e-5):
    m = jnp.mean(x, axis=axis, keepdims=True)
    v = jnp.var(x, axis=axis, keepdims=True)
    return (x - m) / jnp.sqrt(v + eps)
def _scatter_add(tgt, idx, src, axis=0):
    return tgt.at[idx].add(src)
def _segment_sum(src, seg, n):
    return jax.ops.segment_sum(src, seg, n)
class _Rng:
    def __init__(self, key):
        self._k = key
    def _next(self):
        self._k, sub = jax.random.split(self._k)
        return sub
    def normal(self, shape):
        return jax.random.normal(self._next(), shape, dtype=jnp.bfloat16)
    def randint(self, lo, hi, shape):
        return jax.random.randint(self._next(), shape, lo, hi, dtype=jnp.int32)
    def uniform(self, shape, lo=0.0, hi=1.0):
        return jax.random.uniform(self._next(), shape, jnp.bfloat16, lo, hi)
    def permutation(self, n):
        return jax.random.permutation(self._next(), n)


kernel_name = 'gated_mix__gqa_block_cached__dense_activation_relu__decode'

def _fwd_setup_inputs():
    _rng = _Rng(jax.random.key(int.from_bytes(__import__("os").urandom(4), "little")))
    _w = (lambda a: (lambda t: t.astype(jnp.bfloat16) if jnp.issubdtype(t.dtype, jnp.floating) else t)(jnp.asarray(a)))
    def _A_setup():
        B, Sq, D = 2, 1, 512
        Hq, Hkv, Sk, Dh = 32, 8, 8192, 128
        assert Hq % Hkv == 0, (Hq, Hkv)
        return {
            "x": _w((lambda *s: _rng.normal(s) * 0.05)(B, Sq, D)),
            "k_cache": _w((lambda *s: _rng.normal(s) * 0.05)(B, Hkv, Sk, Dh)),
            "v_cache": _w((lambda *s: _rng.normal(s) * 0.05)(B, Hkv, Sk, Dh)),
            "wq": _w((lambda *s: _rng.normal(s) * 0.05)(D, Hq * Dh) * (D ** -0.5)),
            "wo": _w((lambda *s: _rng.normal(s) * 0.05)(Hq * Dh, D) * ((Hq * Dh) ** -0.5)),
        }
    _A_in = _A_setup()

    def _B_setup():
        B, S, D, Dff = 2, 1, 512, 1792
        return {
            "x": _w((lambda *s: _rng.normal(s) * 0.05)(B, S, D)),
            "w1": _w((lambda *s: _rng.normal(s) * 0.05)(D, Dff)),
            "w2": _w((lambda *s: _rng.normal(s) * 0.05)(Dff, D)),
        }
    _B_in = _B_setup()

    return {
        "A_x": _A_in["x"],
        "A_k_cache": _A_in["k_cache"],
        "A_v_cache": _A_in["v_cache"],
        "A_wq": _A_in["wq"],
        "A_wo": _A_in["wo"],
        "B_x": _B_in["x"],
        "B_w1": _B_in["w1"],
        "B_w2": _B_in["w2"],
        "gate_w": _w((lambda *s: _rng.normal(s) * 0.05)(512)),
    }

def _fwd_reference(A_x, A_k_cache, A_v_cache, A_wq, A_wo, B_x, B_w1, B_w2, gate_w):
    def _A_ref(x, k_cache, v_cache, wq, wo):
        B, Sq, D = x.shape
        Hq, Dh = 32, 128
        Hkv = k_cache.shape[1]
        rep = Hq // Hkv
        q = (lambda x, *d: x.transpose(*d))((x @ wq).reshape(B, Sq, Hq, Dh), 0, 2, 1, 3)
        k = jnp.repeat(k_cache, rep, axis=1)
        v = jnp.repeat(v_cache, rep, axis=1)
        scores = jnp.einsum("bhqd,bhkd->bhqk", q, k) * (Dh ** -0.5)
        p = _softmax(scores, axis=-1)
        o = jnp.einsum("bhqk,bhkd->bhqd", p, v)
        return (lambda x, *d: x.transpose(*d))(o, 0, 2, 1, 3).reshape(B, Sq, Hq * Dh) @ wo

    def _B_ref(x, w1, w2):
        h = jnp.einsum("bsd,df->bsf", x, w1)
        zero = jnp.zeros_like(h)
        h = jnp.maximum(h, zero)
        return jnp.einsum("bsf,fd->bsd", h, w2)

    x = A_x
    g = _sigmoid((x * gate_w).sum(-1, keepdims=True))
    a = _A_ref(x, A_k_cache, A_v_cache, A_wq, A_wo)
    b = _B_ref(x, B_w1, B_w2)
    return g * a + (1 - g) * b


def setup_inputs():
    _inp = _fwd_setup_inputs()
    _gk = jax.random.fold_in(jax.random.key(int.from_bytes(__import__("os").urandom(4), "little")), 2**31 - 1)
    _shapes = [[2, 1, 512]]
    _dtypes = ['bfloat16']
    _gks = jax.random.split(_gk, len(_shapes))
    _gs = [jax.random.normal(k, s, dtype=jnp.dtype(d)) * 0.05 for k, s, d in zip(_gks, _shapes, _dtypes)]
    _inp["grad_out"] = _gs[0]
    return _inp

def reference(A_x, A_k_cache, A_v_cache, A_wq, A_wo, B_w1, B_w2, gate_w, B_x, grad_out):
    _const = dict(B_x=B_x)
    def _f(*_d):
        return _fwd_reference(**{'A_x': _d[0], 'A_k_cache': _d[1], 'A_v_cache': _d[2], 'A_wq': _d[3], 'A_wo': _d[4], 'B_w1': _d[5], 'B_w2': _d[6], 'gate_w': _d[7], **_const})
    _out, _vjp = jax.vjp(_f, A_x, A_k_cache, A_v_cache, A_wq, A_wo, B_w1, B_w2, gate_w)
    _grads = _vjp(grad_out)
    _out0 = jnp.asarray(_out)
    return (_out0, *[jnp.asarray(_g) for _g in _grads])
```

```python
import functools
import jax
import jax.numpy as jnp
from jax import lax
import jax.experimental.pallas as pl
import jax.experimental.pallas.tpu as pltpu

F32, BF16 = jnp.float32, jnp.bfloat16
B, D, HQ, HKV, SK, DH, DFF = 2, 512, 32, 8, 8192, 128, 1792
REP = HQ // HKV
NP = B * HKV
HALF = SK // 2
NT = (((1,), (1,)), ((), ()))
TN = (((0,), (0,)), ((), ()))

DEFAULT = dict(
    look=4,
    run=128,
    seg=16,
    first=12,
    step=8,
    switch=15,
    compute=True,
    nobounds=True,
    wpat=1,
)


def make(**kw):
    cfg = dict(DEFAULT)
    cfg.update(kw)
    look, run, seg = cfg["look"], cfg["run"], cfg["seg"]
    nj = HALF // run
    ng = 2 * NP // seg
    n_kv = 2 * ng * nj

    def kernel(x_hbm, k_hbm, v_hbm, wq_hbm, wo_hbm, w1_hbm, w2_hbm, gw_hbm, go_hbm,
               out_hbm, dx_hbm, dk_hbm, dv_hbm, dwq_hbm, dwo_hbm, dw1_hbm, dw2_hbm, dgw_hbm,
               kb, vb, wq, wo, w1, w2, dwq, dwo, dw1, dw2,
               xb, gwb, gob, outb, dxb, dgwb,
               q8_ref, do8_ref, o8_ref, dq8_ref,
               ksem, vsem, rsem, wsem):

        def read_k(p):
            return pltpu.make_async_copy(k_hbm.at[pl.ds(2 * p, 2)], kb.at[pl.ds(2 * p, 2)], ksem.at[p])

        def read_v(p):
            return pltpu.make_async_copy(v_hbm.at[pl.ds(2 * p, 2)], vb.at[pl.ds(2 * p, 2)], vsem.at[p])

        r_wq = pltpu.make_async_copy(wq_hbm, wq, rsem.at[0])
        r_x = pltpu.make_async_copy(x_hbm, xb, rsem.at[1])
        r_gw = pltpu.make_async_copy(gw_hbm, gwb, rsem.at[2])
        r_go = pltpu.make_async_copy(go_hbm, gob, rsem.at[3])
        r_wo = pltpu.make_async_copy(wo_hbm, wo, rsem.at[4])
        r_w1 = pltpu.make_async_copy(w1_hbm, w1, rsem.at[5])
        r_w2 = pltpu.make_async_copy(w2_hbm, w2, rsem.at[6])

        r_wq.start()
        r_x.start()
        r_gw.start()
        r_go.start()
        r_wo.start()

        def start_pair(p, c):
            read_k(p).start()
            read_v(p).start()
        lax.fori_loop(0, look, start_pair, None)

        def write_kv(i):
            g, a, j = i // (2 * nj), (i // nj) % 2, i % nj
            rows = pl.ds(pl.multiple_of(j * run, run), run)
            segs = pl.ds(g * seg, seg)

            @pl.when(a == 0)
            def _():
                pltpu.make_async_copy(kb.at[segs, rows], dk_hbm.at[segs, rows], wsem.at[0]).start()

            @pl.when(a == 1)
            def _():
                pltpu.make_async_copy(vb.at[segs, rows], dv_hbm.at[segs, rows], wsem.at[1]).start()

        def write_kv_range(lo, hi):
            if hi > lo:
                lax.fori_loop(lo, hi, lambda i, c: write_kv(i), None)

        row = lax.broadcasted_iota(jnp.int32, (8, 1), 0)

        def rows8(v):
            return jnp.where(row < REP, v[0:1], v[1:2])

        r_x.wait()
        r_gw.wait()
        r_go.wait()
        x8 = rows8(xb[...].astype(F32))
        go8 = rows8(gob[...].astype(F32))
        gw = gwb[...].astype(F32).reshape(1, D)
        g8 = jax.nn.sigmoid(jnp.sum(x8 * gw, axis=-1, keepdims=True))
        da8 = (g8 * go8).astype(BF16)
        db8 = ((1.0 - g8) * go8).astype(BF16)
        x8b = x8.astype(BF16)

        def head_rows(full, ref):
            for h in range(HKV):
                t = full[:, REP * h * DH:(REP * h + 1) * DH]
                for r in range(1, REP):
                    t = jnp.where(row % REP == r, full[:, (REP * h + r) * DH:(REP * h + r + 1) * DH], t)
                ref[h] = t

        r_wq.wait()
        head_rows(jnp.dot(x8b, wq[...], preferred_element_type=F32), q8_ref)
        r_wo.wait()
        head_rows(lax.dot_general(da8, wo[...], NT, preferred_element_type=F32), do8_ref)

        scale = DH ** -0.5

        def pair(p, c):
            @pl.when(p + look < NP)
            def _():
                read_k(p + look).start()
                read_v(p + look).start()

            @pl.when(p + look == NP)
            def _():
                r_w1.start()
                r_w2.start()

            sw = cfg["switch"]

            @pl.when(p <= sw)
            def _():
                read_k(p).wait()
                read_v(p).wait()

            @pl.when(p == sw)
            def _():
                def wait_pair(i, c):
                    read_k(i).wait()
                    read_v(i).wait()
                if sw + 1 < NP:
                    lax.fori_loop(sw + 1, NP, wait_pair, None)
                r_w1.wait()
                r_w2.wait()
                write_kv_range(0, cfg["first"])

            if not cfg["compute"]:
                return
            b, h = p // HKV, p % HKV

            def both(t):
                u = pltpu.roll(t, REP, 0)
                return jnp.where((row < REP) == (b == 0), t, u)

            qq = both(q8_ref[h]).astype(BF16)
            dd = both(do8_ref[h]).astype(BF16)
            s = jnp.concatenate(
                [lax.dot_general(qq, kb[2 * p + i], NT, preferred_element_type=F32) for i in range(2)],
                axis=1) * scale
            dp = jnp.concatenate(
                [lax.dot_general(dd, vb[2 * p + i], NT, preferred_element_type=F32) for i in range(2)],
                axis=1)
            e = jnp.exp(s - jnp.max(s, axis=-1, keepdims=True))
            prob = e * (1.0 / jnp.sum(e, axis=-1, keepdims=True))
            delta = jnp.sum(prob * dp, axis=-1, keepdims=True)
            ds = prob * (dp - delta) * scale
            pd = jnp.where(row < REP, ds, prob)
            pdb = pd.astype(BF16)
            dq = sum(jnp.dot(pdb[:, i * HALF:(i + 1) * HALF], kb[2 * p + i], preferred_element_type=F32)
                     for i in range(2))
            o = sum(jnp.dot(pdb[:, i * HALF:(i + 1) * HALF], vb[2 * p + i], preferred_element_type=F32)
                    for i in range(2))
            dq8_ref[b, h] = dq
            o8_ref[b, h] = o

            nb = 128 // 8
            blk = SK // nb
            pdt = jnp.concatenate([pd[:, j * blk:(j + 1) * blk] for j in range(nb)], axis=0).T.astype(BF16)
            wk = jnp.tile(jnp.where(row < REP, qq.astype(F32), 0.0), (nb, 1))
            wv = jnp.tile(jnp.where(row < REP, 0.0, dd.astype(F32)), (nb, 1))
            grp = lax.broadcasted_iota(jnp.int32, (128, DH), 0) // 8
            for j in range(nb):
                i, r0 = divmod(j * blk, HALF)
                kb[2 * p + i, r0:r0 + blk] = jnp.dot(
                    pdt, jnp.where(grp == j, wk, 0.0).astype(BF16), preferred_element_type=F32).astype(BF16)
                vb[2 * p + i, r0:r0 + blk] = jnp.dot(
                    pdt, jnp.where(grp == j, wv, 0.0).astype(BF16), preferred_element_type=F32).astype(BF16)

        lax.fori_loop(0, NP, pair, None)

        done = cfg["first"]
        step = cfg["step"]
        write_kv_range(done, done + step)
        done += step

        first = row % REP == 0
        hpre = jnp.dot(x8b, w1[...], preferred_element_type=F32).astype(BF16).astype(F32)
        act = jnp.maximum(hpre, 0.0).astype(BF16)
        b8 = jnp.dot(act, w2[...], preferred_element_type=F32)
        slope = jnp.where(hpre > 0.0, 1.0, jnp.where(hpre == 0.0, 0.5, 0.0))
        dh = (lax.dot_general(db8, w2[...], NT, preferred_element_type=F32) * slope).astype(BF16)
        dx8 = lax.dot_general(dh, w1[...], NT, preferred_element_type=F32)
        x1 = jnp.where(first, x8, 0.0).astype(BF16)
        db1 = jnp.where(first, db8.astype(F32), 0.0).astype(BF16)
        dw1[...] = lax.dot_general(x1, dh, TN, preferred_element_type=F32).astype(BF16).reshape(dw1.shape)
        dw2[...] = lax.dot_general(act, db1, TN, preferred_element_type=F32).astype(BF16).reshape(dw2.shape)

        write_kv_range(done, done + step)
        done += step

        def head_cols(ref, hi):
            cols = []
            for h in range(HKV):
                t0, t1 = ref[0, h], ref[1, h]
                if hi:
                    t = jnp.where(row < REP, pltpu.roll(t0, REP, 0), t1)
                else:
                    t = jnp.where(row < REP, t0, pltpu.roll(t1, REP, 0))
                cols += [jnp.where(row % REP == r, t, 0.0) for r in range(REP)]
            return jnp.concatenate(cols, axis=1).astype(BF16)

        def batch_sum(t):
            return jnp.where(row < REP, jnp.sum(t[:REP], axis=0, keepdims=True),
                             jnp.sum(t[REP:], axis=0, keepdims=True))

        of = head_cols(o8_ref, True)
        a8 = batch_sum(jnp.dot(of, wo[...], preferred_element_type=F32))
        dwo[...] = lax.dot_general(of, da8, TN, preferred_element_type=F32).astype(BF16).reshape(dwo.shape)

        write_kv_range(done, done + step)
        done += step

        dqf = head_cols(dq8_ref, False)
        dx8 = dx8 + batch_sum(lax.dot_general(dqf, wq[...], NT, preferred_element_type=F32))
        dwq[...] = lax.dot_general(x8b, dqf, TN, preferred_element_type=F32).astype(BF16).reshape(dwq.shape)

        dz8 = jnp.sum(go8 * (a8 - b8), axis=-1, keepdims=True) * g8 * (1.0 - g8)
        out8 = g8 * a8 + (1.0 - g8) * b8
        dx8 = dx8 + dz8 * gw
        two = lax.broadcasted_iota(jnp.int32, (2, 1), 0) == 0
        outb[...] = jnp.where(two, out8[0:1], out8[REP:REP + 1]).astype(BF16)
        dxb[...] = jnp.where(two, dx8[0:1], dx8[REP:REP + 1]).astype(BF16)
        t = dz8 * x8
        dgwb[...] = (t[0:1] + t[REP:REP + 1]).astype(BF16).reshape(D)

        small = [pltpu.make_async_copy(outb, out_hbm, wsem.at[6]),
                 pltpu.make_async_copy(dxb, dx_hbm, wsem.at[7]),
                 pltpu.make_async_copy(dgwb, dgw_hbm, wsem.at[8])]
        for c in small:
            c.start()

        def write_w(src, dst, sem, n, rows, cols=None):
            def one(j, c):
                if cols is None:
                    r = pl.ds(pl.multiple_of(j * rows, rows), rows)
                    pltpu.make_async_copy(src.at[:, r], dst.at[:, r], sem).start()
                else:
                    per = src.shape[2] // cols
                    r = pl.ds(pl.multiple_of((j // per) * rows, rows), rows)
                    cc = pl.ds(pl.multiple_of((j % per) * cols, cols), cols)
                    pltpu.make_async_copy(src.at[:, r, cc], dst.at[:, r, cc], sem).start()
            lax.fori_loop(0, n, one, None)

        if cfg["wpat"] == 0:
            for s_, d_, i_ in ((dwq, dwq_hbm, 2), (dwo, dwo_hbm, 3), (dw1, dw1_hbm, 4), (dw2, dw2_hbm, 5)):
                pltpu.make_async_copy(s_, d_, wsem.at[i_]).start()
        else:
            write_w(dwq, dwq_hbm, wsem.at[2], 16, 16, 1024)
            write_w(dwo, dwo_hbm, wsem.at[3], 16, 32)
            write_w(dw1, dw1_hbm, wsem.at[4], 8, 16)
            write_w(dw2, dw2_hbm, wsem.at[5], 14, 32)

        write_kv_range(done, n_kv)

        for c in small:
            c.wait()
        pltpu.make_async_copy(dwq, dwq_hbm, wsem.at[2]).wait()
        pltpu.make_async_copy(dwo, dwo_hbm, wsem.at[3]).wait()
        pltpu.make_async_copy(dw1, dw1_hbm, wsem.at[4]).wait()
        pltpu.make_async_copy(dw2, dw2_hbm, wsem.at[5]).wait()
        pltpu.make_async_copy(kb, dk_hbm, wsem.at[0]).wait()
        pltpu.make_async_copy(vb, dv_hbm, wsem.at[1]).wait()

    kv_shape = (2 * NP, HALF, DH)
    wq_s, wo_s, w1_s, w2_s = (8, D // 8, HQ * DH), (8, HQ * DH // 8, D), (4, D // 4, DFF), (4, DFF // 4, D)
    hbm = pl.BlockSpec(memory_space=pltpu.HBM)
    sds = jax.ShapeDtypeStruct

    def run_fn(A_x, A_k_cache, A_v_cache, A_wq, A_wo, B_x, B_w1, B_w2, gate_w, grad_out):
        outs = pl.pallas_call(
            kernel,
            in_specs=[hbm] * 9,
            out_specs=[hbm] * 9,
            out_shape=[sds((B, D), BF16), sds((B, D), BF16), sds(kv_shape, BF16), sds(kv_shape, BF16),
                       sds(wq_s, BF16), sds(wo_s, BF16), sds(w1_s, BF16), sds(w2_s, BF16), sds((D,), BF16)],
            scratch_shapes=[
                pltpu.VMEM(kv_shape, BF16), pltpu.VMEM(kv_shape, BF16),
                pltpu.VMEM((D, HQ * DH), BF16), pltpu.VMEM((HQ * DH, D), BF16),
                pltpu.VMEM((D, DFF), BF16), pltpu.VMEM((DFF, D), BF16),
                pltpu.VMEM(wq_s, BF16), pltpu.VMEM(wo_s, BF16), pltpu.VMEM(w1_s, BF16), pltpu.VMEM(w2_s, BF16),
                pltpu.VMEM((B, D), BF16), pltpu.VMEM((D,), BF16), pltpu.VMEM((B, D), BF16),
                pltpu.VMEM((B, D), BF16), pltpu.VMEM((B, D), BF16), pltpu.VMEM((D,), BF16),
                pltpu.VMEM((HKV, 8, DH), F32), pltpu.VMEM((HKV, 8, DH), F32),
                pltpu.VMEM((B, HKV, 8, DH), F32), pltpu.VMEM((B, HKV, 8, DH), F32),
                pltpu.SemaphoreType.DMA((NP,)), pltpu.SemaphoreType.DMA((NP,)),
                pltpu.SemaphoreType.DMA((7,)), pltpu.SemaphoreType.DMA((9,)),
            ],
            compiler_params=pltpu.CompilerParams(
                vmem_limit_bytes=120 * 1024 * 1024, disable_bounds_checks=cfg["nobounds"]),
        )(A_x.reshape(B, D), A_k_cache.reshape(kv_shape), A_v_cache.reshape(kv_shape), A_wq, A_wo,
          B_w1, B_w2, gate_w, grad_out.reshape(B, D))
        out, dx, dk, dv, dwq, dwo, dw1, dw2, dgw = outs
        return (out.reshape(B, 1, D), dx.reshape(B, 1, D),
                dk.reshape(A_k_cache.shape), dv.reshape(A_v_cache.shape),
                dwq.reshape(A_wq.shape), dwo.reshape(A_wo.shape),
                dw1.reshape(B_w1.shape), dw2.reshape(B_w2.shape), dgw)

    return run_fn


_impl = make()


@jax.jit
def pallas_gated_mix__gqa_block_cached__dense_activation_relu__decode_kernel(
    A_x, A_k_cache, A_v_cache, A_wq, A_wo, B_x, B_w1, B_w2, gate_w, grad_out):
    return _impl(A_x, A_k_cache, A_v_cache, A_wq, A_wo, B_x, B_w1, B_w2, gate_w, grad_out)
```

```python
import functools

import jax
import jax.numpy as jnp
from jax import lax
import jax.experimental.pallas as pl
import jax.experimental.pallas.tpu as pltpu

F32, BF16 = jnp.float32, jnp.bfloat16
B, D, HQ, HKV, SK, DH, DFF = 2, 512, 32, 8, 8192, 128, 1792
REP = HQ // HKV
NPAIR = B * HKV
NT = (((1,), (1,)), ((), ()))
TN = (((0,), (0,)), ((), ()))

HALF = SK // 2
KV_SHAPE = (2 * NPAIR, HALF, DH)
WQ_SHAPE, WO_SHAPE = (4, D // 4, HQ * DH), (4, HQ * DH // 4, D)
W1_SHAPE, W2_SHAPE = (2, D // 2, DFF), (2, DFF // 2, D)

READ_STREAMS, READ_ROWS = 2 * HKV, 16
READ_URGENT = 2
STEP_ROUNDS = 4
PART_STEPS = HALF // (READ_ROWS * STEP_ROUNDS)
LOOK_AHEAD = 8
PROLOGUE_STEPS = 8
POINT_STEPS = 5
TAIL_STEPS = 1
SWITCH = -(-(2 * PART_STEPS - LOOK_AHEAD) // (4 * POINT_STEPS))

WRITE_GROUPS, WRITE_ROWS = ((0, 6), (6, 6), (12, 6), (18, 7), (25, 7)), 64
PART_WRITES = HALF // WRITE_ROWS
ALL_WRITES = 2 * len(WRITE_GROUPS) * PART_WRITES
EARLY_WRITES, FIRST_WRITES, PAIR_WRITES = 8, 72, 52


def _writes_before(p):
    ready = sum(2 * PART_WRITES for at, n in WRITE_GROUPS if at + n <= 2 * p)
    return min(FIRST_WRITES + (p - SWITCH) * PAIR_WRITES, ready)


def _copy(src, dst, sem, *idx):
    return pltpu.make_async_copy(src.at[idx], dst.at[idx], sem)


def _block(i, n):
    return pl.ds(pl.multiple_of(i * n, n), n)


def _loop(lo, hi, body):
    if isinstance(lo, int) and isinstance(hi, int) and hi <= lo:
        return
    lax.fori_loop(lo, hi, lambda i, carry: body(i), None)


def _clip(v, lo, hi):
    return min(max(v, lo), hi) if isinstance(v, int) else jnp.clip(v, lo, hi)


def _dot(a, b, dims=(((1,), (0,)), ((), ()))):
    return lax.dot_general(a, b, dims, preferred_element_type=F32)


def _kernel(x_hbm, k_hbm, v_hbm, wq_hbm, wo_hbm, w1_hbm, w2_hbm, gw_hbm, go_hbm,
            out_hbm, dx_hbm, dk_hbm, dv_hbm, dwq_hbm, dwo_hbm, dw1_hbm, dw2_hbm, dgw_hbm,
            k_ref, v_ref, wq_ref, wo_ref, w1_ref, w2_ref, dwq_ref, dwo_ref, dw1_ref, dw2_ref,
            x_ref, gw_ref, go_ref, out_ref, dx_ref, dgw_ref,
            q_ref, do_ref, o_ref, dq_ref, sems):
    sem_q, sem_o, sem_1, sem_2, sem_small, sem_k, sem_v = (sems.at[i] for i in range(7))
    part_sems, sem_tail = (sem_k, sem_v, sem_q, sem_o), sem_1

    def read_weights(with_mlp, j):
        half = _block(j >> 1, 8), _block(j & 1, 256)
        _copy(wq_hbm, wq_ref, sem_q, pl.ds(0, 4), _block(j >> 4, 8), _block(j & 15, 256)).start(priority=1)
        if with_mlp:
            _copy(wo_hbm, wo_ref, sem_o, pl.ds(0, 4), *half).start(priority=1)
            _copy(w1_hbm, w1_ref, sem_1, pl.ds(0, 2), _block(j // 7, 8), _block(j % 7, 256)).start(priority=1)
            _copy(w2_hbm, w2_ref, sem_2, pl.ds(0, 2), *half).start(priority=0)
        else:
            _copy(wo_hbm, wo_ref, sem_o, pl.ds(0, 3), *half).start(priority=1)
            _copy(wo_hbm, wo_ref, sem_o, pl.ds(3, 1), *half).start(priority=0)

    def part_refs(c):
        return ((k_hbm, k_ref), (v_hbm, v_ref))[c % 2], c // 2 * READ_STREAMS

    def read_step(c, sem, j):
        (src, dst), at = part_refs(c)
        bulk = READ_STREAMS - READ_URGENT
        for u in range(STEP_ROUNDS):
            rows = _block(j * STEP_ROUNDS + u, READ_ROWS)
            _copy(src, dst, sem, pl.ds(at, bulk), rows).start(priority=1)
            _copy(src, dst, sem, pl.ds(at + bulk, READ_URGENT), rows).start(priority=0)

    def read_steps(lo, hi, parts=(0, 1, 2)):
        for c in parts:
            lo_c, hi_c = lo - c * PART_STEPS, hi - c * PART_STEPS
            end = PART_STEPS - (TAIL_STEPS if c == 3 else 0)
            _loop(_clip(lo_c, 0, end), _clip(hi_c, 0, end), functools.partial(read_step, c, part_sems[c]))
            if end < PART_STEPS:
                _loop(_clip(lo_c, end, PART_STEPS), _clip(hi_c, end, PART_STEPS),
                      functools.partial(read_step, c, sem_tail))

    def wait_part(c, sem, row=0, rows=HALF):
        (src, dst), at = part_refs(c)
        _copy(src, dst, sem, pl.ds(at, READ_STREAMS), pl.ds(row, rows)).wait()

    def write_cache(c, j):
        src, dst, sem = ((k_ref, dk_hbm, sem_k), (v_ref, dv_hbm, sem_v))[c % 2]
        _copy(src, dst, sem, pl.ds(*WRITE_GROUPS[c // 2]), _block(j, WRITE_ROWS)).start()

    def write_caches(lo, hi):
        for c in range(2 * len(WRITE_GROUPS)):
            _loop(_clip(lo - c * PART_WRITES, 0, PART_WRITES), _clip(hi - c * PART_WRITES, 0, PART_WRITES),
                  functools.partial(write_cache, c))

    def write_wq_w1(j):
        _copy(dwq_ref, dwq_hbm, sem_q, pl.ds(0, 4), _block(j >> 2, 8), _block(j & 3, 1024)).start()
        _copy(dw1_ref, dw1_hbm, sem_1, pl.ds(0, 2), _block(j >> 1, 8), _block(j & 1, 896)).start()

    def write_wo_w2(with_mlp, j):
        _copy(dwo_ref, dwo_hbm, sem_o, pl.ds(0, 4), _block(j, 16)).start()
        if with_mlp:
            _copy(dw2_ref, dw2_hbm, sem_2, pl.ds(0, 2), _block(j, 16)).start()

    small_in = [pltpu.make_async_copy(src, dst, sem_small)
                for src, dst in ((x_hbm, x_ref), (gw_hbm, gw_ref), (go_hbm, go_ref))]
    _loop(0, 224, functools.partial(read_weights, True))
    for c in small_in:
        c.start()
    _loop(224, 256, functools.partial(read_weights, False))
    read_steps(0, LOOK_AHEAD)

    stage = [LOOK_AHEAD]

    def prologue_reads():
        read_steps(stage[0], stage[0] + PROLOGUE_STEPS)
        stage[0] += PROLOGUE_STEPS

    row = lax.broadcasted_iota(jnp.int32, (8, 1), 0)
    low = row < REP

    def tile(ref):
        v = ref[...].astype(F32)
        return jnp.where(low, v[0:1], v[1:2])

    def matrix(ref):
        return ref[...].reshape(-1, ref.shape[-1])

    def store_heads(full, ref):
        for h in range(HKV):
            t = full[:, REP * h * DH:(REP * h + 1) * DH]
            for r in range(1, REP):
                t = jnp.where(row % REP == r, full[:, (REP * h + r) * DH:(REP * h + r + 1) * DH], t)
            ref[h] = t

    for c in small_in:
        c.wait()
    x, go = tile(x_ref), tile(go_ref)
    gw = gw_ref[...].astype(F32).reshape(1, D)
    gate = jax.nn.sigmoid(jnp.sum(x * gw, axis=-1, keepdims=True))
    da = (gate * go).astype(BF16)
    db = ((1.0 - gate) * go).astype(BF16)
    xb = x.astype(BF16)

    pltpu.make_async_copy(w1_hbm, w1_ref, sem_1).wait()
    pltpu.make_async_copy(w2_hbm, w2_ref, sem_2).wait()
    pltpu.make_async_copy(wq_hbm, wq_ref, sem_q).wait()
    pltpu.make_async_copy(wo_hbm, wo_ref, sem_o).wait()
    prologue_reads()
    store_heads(_dot(xb, matrix(wq_ref)), q_ref)
    prologue_reads()
    store_heads(_dot(da, matrix(wo_ref), NT), do_ref)
    prologue_reads()

    h_pre = _dot(xb, matrix(w1_ref)).astype(BF16).astype(F32)
    act = jnp.maximum(h_pre, 0.0).astype(BF16)
    mlp = _dot(act, matrix(w2_ref))
    slope = jnp.where(h_pre > 0.0, 1.0, jnp.where(h_pre == 0.0, 0.5, 0.0))
    dh = (_dot(db, matrix(w2_ref), NT) * slope).astype(BF16)
    dx = _dot(dh, matrix(w1_ref), NT)
    prologue_reads()
    once = row % REP == 0
    dw1_ref[...] = _dot(jnp.where(once, x, 0.0).astype(BF16), dh, TN).astype(BF16).reshape(W1_SHAPE)
    prologue_reads()
    dw2_ref[...] = _dot(act, jnp.where(once, db.astype(F32), 0.0).astype(BF16), TN).astype(BF16).reshape(W2_SHAPE)
    read_steps(stage[0], 2 * PART_STEPS + LOOK_AHEAD)
    wait_part(0, part_sems[0])
    wait_part(1, part_sems[1])

    scale = DH ** -0.5

    def pair(p):
        @pl.when(p == SWITCH)
        def _():
            tail = TAIL_STEPS * STEP_ROUNDS * READ_ROWS
            wait_part(2, part_sems[2])
            wait_part(3, part_sems[3], 0, HALF - tail)
            write_caches(0, EARLY_WRITES)
            wait_part(3, sem_tail, HALF - tail, tail)
            write_caches(EARLY_WRITES, _writes_before(SWITCH))

        for i in range(SWITCH + 1, NPAIR):
            pl.when(p == i)(functools.partial(write_caches, _writes_before(i - 1), _writes_before(i)))

        def reads(i):
            @pl.when(p < SWITCH)
            def _():
                lo = 2 * PART_STEPS + LOOK_AHEAD + (4 * p + i) * POINT_STEPS
                read_steps(lo, lo + POINT_STEPS, (2, 3))

        reads(0)
        b, h = p // HKV, p % HKV

        def own_rows(t):
            return jnp.where(low == (b == 0), t, pltpu.roll(t, REP, 0)).astype(BF16)

        q, do = own_rows(q_ref[h]), own_rows(do_ref[h])
        s = jnp.concatenate([_dot(q, k_ref[2 * p + i], NT) for i in range(2)], axis=1) * scale
        dp = jnp.concatenate([_dot(do, v_ref[2 * p + i], NT) for i in range(2)], axis=1)
        e = jnp.exp(s - jnp.max(s, axis=-1, keepdims=True))
        prob = e * (1.0 / jnp.sum(e, axis=-1, keepdims=True))
        ds = prob * (dp - jnp.sum(prob * dp, axis=-1, keepdims=True)) * scale
        both = jnp.where(low, ds, prob)
        both_b = both.astype(BF16)
        reads(1)
        dq_ref[b, h] = sum(_dot(both_b[:, i * HALF:(i + 1) * HALF], k_ref[2 * p + i]) for i in range(2))
        o_ref[b, h] = sum(_dot(both_b[:, i * HALF:(i + 1) * HALF], v_ref[2 * p + i]) for i in range(2))

        blocks = 128 // 8
        rows = SK // blocks
        folded = jnp.concatenate([both[:, j * rows:(j + 1) * rows] for j in range(blocks)], axis=0)
        folded = folded.T.astype(BF16)
        for_k = jnp.tile(jnp.where(low, q.astype(F32), 0.0), (blocks, 1))
        for_v = jnp.tile(jnp.where(low, 0.0, do.astype(F32)), (blocks, 1))
        block = lax.broadcasted_iota(jnp.int32, (128, DH), 0) // 8
        for j in range(blocks):
            if j in (3, 9):
                reads(2 + j // 8)
            i, at = divmod(j * rows, HALF)
            k_ref[2 * p + i, at:at + rows] = _dot(folded, jnp.where(block == j, for_k, 0.0).astype(BF16)).astype(BF16)
            v_ref[2 * p + i, at:at + rows] = _dot(folded, jnp.where(block == j, for_v, 0.0).astype(BF16)).astype(BF16)

    _loop(0, NPAIR, pair)

    def spread_heads(ref, high):
        cols = []
        for h in range(HKV):
            t0, t1 = ref[0, h], ref[1, h]
            if high:
                t = jnp.where(low, pltpu.roll(t0, REP, 0), t1)
            else:
                t = jnp.where(low, t0, pltpu.roll(t1, REP, 0))
            cols += [jnp.where(row % REP == r, t, 0.0) for r in range(REP)]
        return jnp.concatenate(cols, axis=1).astype(BF16)

    def per_token(t):
        return jnp.where(low, jnp.sum(t[:REP], axis=0, keepdims=True), jnp.sum(t[REP:], axis=0, keepdims=True))

    queued = _writes_before(NPAIR - 1)
    write_caches(queued, queued + PAIR_WRITES)
    o = spread_heads(o_ref, True)
    attn = per_token(_dot(o, matrix(wo_ref)))
    dwo_ref[...] = _dot(o, da, TN).astype(BF16).reshape(WO_SHAPE)

    write_caches(queued + PAIR_WRITES, queued + 2 * PAIR_WRITES)
    dq = spread_heads(dq_ref, False)
    dx = dx + per_token(_dot(dq, matrix(wq_ref), NT))
    dwq_ref[...] = _dot(xb, dq, TN).astype(BF16).reshape(WQ_SHAPE)

    dz = jnp.sum(go * (attn - mlp), axis=-1, keepdims=True) * gate * (1.0 - gate)
    out = gate * attn + (1.0 - gate) * mlp
    dx = dx + dz * gw
    dgw = dz * x
    token0 = lax.broadcasted_iota(jnp.int32, (B, 1), 0) == 0
    out_ref[...] = jnp.where(token0, out[0:1], out[REP:REP + 1]).astype(BF16)
    dx_ref[...] = jnp.where(token0, dx[0:1], dx[REP:REP + 1]).astype(BF16)
    dgw_ref[...] = (dgw[0:1] + dgw[REP:REP + 1]).astype(BF16).reshape(D)

    write_caches(queued + 2 * PAIR_WRITES, ALL_WRITES)
    small_out = [pltpu.make_async_copy(src, dst, sem_small)
                 for src, dst in ((out_ref, out_hbm), (dx_ref, dx_hbm), (dgw_ref, dgw_hbm))]
    for c in small_out:
        c.start()
    _loop(0, 64, write_wq_w1)
    _loop(0, 56, functools.partial(write_wo_w2, True))
    _loop(56, 64, functools.partial(write_wo_w2, False))

    for c in small_out:
        c.wait()
    for src, dst, sem in ((k_ref, dk_hbm, sem_k), (v_ref, dv_hbm, sem_v), (dwq_ref, dwq_hbm, sem_q),
                          (dw1_ref, dw1_hbm, sem_1), (dw2_ref, dw2_hbm, sem_2), (dwo_ref, dwo_hbm, sem_o)):
        pltpu.make_async_copy(src, dst, sem).wait()


@jax.jit
def pallas_gated_mix__gqa_block_cached__dense_activation_relu__decode_kernel(
    A_x: jax.Array,
    A_k_cache: jax.Array,
    A_v_cache: jax.Array,
    A_wq: jax.Array,
    A_wo: jax.Array,
    B_x: jax.Array,
    B_w1: jax.Array,
    B_w2: jax.Array,
    gate_w: jax.Array,
    grad_out: jax.Array,
):
    del B_x
    weights = (WQ_SHAPE, WO_SHAPE, W1_SHAPE, W2_SHAPE)
    token, vector = (B, D), (D,)
    hbm = pl.BlockSpec(memory_space=pltpu.HBM)
    out, dx, dk, dv, dwq, dwo, dw1, dw2, dgw = pl.pallas_call(
        _kernel,
        in_specs=[hbm] * 9,
        out_specs=[hbm] * 9,
        out_shape=[jax.ShapeDtypeStruct(s, BF16) for s in (token, token, KV_SHAPE, KV_SHAPE, *weights, vector)],
        scratch_shapes=[
            *(pltpu.VMEM(s, BF16) for s in (KV_SHAPE, KV_SHAPE, *weights, *weights)),
            *(pltpu.VMEM(s, BF16) for s in (token, vector, token, token, token, vector)),
            pltpu.VMEM((HKV, 8, DH), F32), pltpu.VMEM((HKV, 8, DH), F32),
            pltpu.VMEM((B, HKV, 8, DH), F32), pltpu.VMEM((B, HKV, 8, DH), F32),
            pltpu.SemaphoreType.DMA((7,)),
        ],
        compiler_params=pltpu.CompilerParams(vmem_limit_bytes=120 * 1024 * 1024, disable_bounds_checks=True),
    )(A_x.reshape(token), A_k_cache.reshape(KV_SHAPE), A_v_cache.reshape(KV_SHAPE),
      A_wq.reshape(WQ_SHAPE), A_wo.reshape(WO_SHAPE), B_w1.reshape(W1_SHAPE), B_w2.reshape(W2_SHAPE),
      gate_w, grad_out.reshape(token))
    return (out.reshape(A_x.shape), dx.reshape(A_x.shape), dk.reshape(A_k_cache.shape), dv.reshape(A_v_cache.shape),
            dwq.reshape(A_wq.shape), dwo.reshape(A_wo.shape), dw1.reshape(B_w1.shape), dw2.reshape(B_w2.shape), dgw)
```

```python
import functools

import jax
import jax.numpy as jnp
from jax import lax
import jax.experimental.pallas as pl
import jax.experimental.pallas.tpu as pltpu

F32, BF16 = jnp.float32, jnp.bfloat16
B, D, HQ, HKV, SK, DH, DFF = 2, 512, 32, 8, 8192, 128, 1792
REP = HQ // HKV
NPAIR = B * HKV
NT = (((1,), (1,)), ((), ()))
TN = (((0,), (0,)), ((), ()))

HALF = SK // 2
KV_SHAPE = (2 * NPAIR, HALF, DH)
WQ_SHAPE, WO_SHAPE = (4, D // 4, HQ * DH), (4, HQ * DH // 4, D)
W1_SHAPE, W2_SHAPE = (2, D // 2, DFF), (2, DFF // 2, D)

READ_STREAMS, READ_ROWS = 2 * HKV, 16
READ_URGENT = 2
STEP_ROUNDS = 4
PART_STEPS = HALF // (READ_ROWS * STEP_ROUNDS)
LOOK_AHEAD = 8
PROLOGUE_STEPS = 8
POINT_STEPS = 5
LAST_STEPS = 2
LAST_SPLIT = (3, 1)
TAIL_ROUNDS = 7
SWITCH = -(-(2 * PART_STEPS - LOOK_AHEAD - LAST_STEPS) // (4 * POINT_STEPS))

assert SWITCH <= HKV and TAIL_ROUNDS <= LAST_STEPS * STEP_ROUNDS

WRITE_GROUPS, WRITE_ROWS = ((0, 6), (6, 6), (12, 6), (18, 7), (25, 7)), 64
PART_WRITES = HALF // WRITE_ROWS
ALL_WRITES = 2 * len(WRITE_GROUPS) * PART_WRITES
EARLY_WRITES, FIRST_WRITES, PAIR_WRITES = 8, 72, 52


def _writes_before(p):
    ready = sum(2 * PART_WRITES for at, n in WRITE_GROUPS if at + n <= 2 * p)
    return min(FIRST_WRITES + (p - SWITCH) * PAIR_WRITES, ready)


def _copy(src, dst, sem, *idx):
    return pltpu.make_async_copy(src.at[idx], dst.at[idx], sem)


def _block(i, n):
    return pl.ds(pl.multiple_of(i * n, n), n)


def _loop(lo, hi, body):
    if isinstance(lo, int) and isinstance(hi, int) and hi <= lo:
        return
    lax.fori_loop(lo, hi, lambda i, carry: body(i), None)


def _clip(v, lo, hi):
    return min(max(v, lo), hi) if isinstance(v, int) else jnp.clip(v, lo, hi)


def _dot(a, b, dims=(((1,), (0,)), ((), ()))):
    return lax.dot_general(a, b, dims, preferred_element_type=F32)


def _kernel(x_hbm, k_hbm, v_hbm, wq_hbm, wo_hbm, w1_hbm, w2_hbm, gw_hbm, go_hbm,
            out_hbm, dx_hbm, dk_hbm, dv_hbm, dwq_hbm, dwo_hbm, dw1_hbm, dw2_hbm, dgw_hbm,
            k_ref, v_ref, wq_ref, wo_ref, w1_ref, w2_ref, dwq_ref, dwo_ref, dw1_ref, dw2_ref,
            x_ref, gw_ref, go_ref, out_ref, dx_ref, dgw_ref,
            q_ref, do_ref, o_ref, dq_ref, sems):
    sem_q, sem_o, sem_1, sem_2, sem_small, sem_k, sem_v = (sems.at[i] for i in range(7))
    part_sems, sem_tail = (sem_k, sem_v, sem_q, sem_o), sem_1

    def read_weights(with_mlp, j):
        half = _block(j >> 1, 8), _block(j & 1, 256)
        _copy(wq_hbm, wq_ref, sem_q, pl.ds(0, 4), _block(j >> 4, 8), _block(j & 15, 256)).start(priority=1)
        if with_mlp:
            _copy(wo_hbm, wo_ref, sem_o, pl.ds(0, 4), *half).start(priority=1)
            _copy(w1_hbm, w1_ref, sem_1, pl.ds(0, 2), _block(j // 7, 8), _block(j % 7, 256)).start(priority=1)
            _copy(w2_hbm, w2_ref, sem_2, pl.ds(0, 2), *half).start(priority=0)
        else:
            _copy(wo_hbm, wo_ref, sem_o, pl.ds(0, 3), *half).start(priority=1)
            _copy(wo_hbm, wo_ref, sem_o, pl.ds(3, 1), *half).start(priority=0)

    def part_refs(c):
        return ((k_hbm, k_ref), (v_hbm, v_ref))[c % 2], c // 2 * READ_STREAMS

    def read_round(c, sem, rows, split):
        (src, dst), first = part_refs(c)
        for at in range(first, first + READ_STREAMS, sum(split)):
            _copy(src, dst, sem, pl.ds(at, split[0]), rows).start(priority=1)
            _copy(src, dst, sem, pl.ds(at + split[0], split[1]), rows).start(priority=0)

    def read_step(c, j):
        for u in range(STEP_ROUNDS):
            read_round(c, part_sems[c], _block(j * STEP_ROUNDS + u, READ_ROWS),
                       (READ_STREAMS - READ_URGENT, READ_URGENT))

    def read_steps(lo, hi, parts=(0, 1, 2)):
        for c in parts:
            end = PART_STEPS - (LAST_STEPS if c == 3 else 0)
            _loop(_clip(lo - c * PART_STEPS, 0, end), _clip(hi - c * PART_STEPS, 0, end),
                  functools.partial(read_step, c))

    def read_last_steps():
        rounds = PART_STEPS * STEP_ROUNDS
        for lo, hi, sem in ((rounds - LAST_STEPS * STEP_ROUNDS, rounds - TAIL_ROUNDS, part_sems[3]),
                            (rounds - TAIL_ROUNDS, rounds, sem_tail)):
            _loop(lo, hi, lambda j, sem=sem: read_round(3, sem, _block(j, READ_ROWS), LAST_SPLIT))

    def wait_part(c, sem, row=0, rows=HALF):
        (src, dst), at = part_refs(c)
        _copy(src, dst, sem, pl.ds(at, READ_STREAMS), pl.ds(row, rows)).wait()

    def write_cache(c, j):
        src, dst, sem = ((k_ref, dk_hbm, sem_k), (v_ref, dv_hbm, sem_v))[c % 2]
        _copy(src, dst, sem, pl.ds(*WRITE_GROUPS[c // 2]), _block(j, WRITE_ROWS)).start()

    def write_caches(lo, hi):
        for c in range(2 * len(WRITE_GROUPS)):
            _loop(_clip(lo - c * PART_WRITES, 0, PART_WRITES), _clip(hi - c * PART_WRITES, 0, PART_WRITES),
                  functools.partial(write_cache, c))

    def write_wq_w1(j):
        _copy(dwq_ref, dwq_hbm, sem_q, pl.ds(0, 4), _block(j >> 2, 8), _block(j & 3, 1024)).start()
        _copy(dw1_ref, dw1_hbm, sem_1, pl.ds(0, 2), _block(j >> 1, 8), _block(j & 1, 896)).start()

    def write_wo_w2(with_mlp, j):
        _copy(dwo_ref, dwo_hbm, sem_o, pl.ds(0, 4), _block(j, 16)).start()
        if with_mlp:
            _copy(dw2_ref, dw2_hbm, sem_2, pl.ds(0, 2), _block(j, 16)).start()

    small_in = [pltpu.make_async_copy(src, dst, sem_small)
                for src, dst in ((x_hbm, x_ref), (gw_hbm, gw_ref), (go_hbm, go_ref))]
    _loop(0, 224, functools.partial(read_weights, True))
    for c in small_in:
        c.start()
    _loop(224, 256, functools.partial(read_weights, False))
    read_steps(0, LOOK_AHEAD)

    stage = [LOOK_AHEAD]

    def prologue_reads():
        read_steps(stage[0], stage[0] + PROLOGUE_STEPS)
        stage[0] += PROLOGUE_STEPS

    row = lax.broadcasted_iota(jnp.int32, (8, 1), 0)
    low = row < REP

    def tile(ref):
        v = ref[...].astype(F32)
        return jnp.where(low, v[0:1], v[1:2])

    def matrix(ref):
        return ref[...].reshape(-1, ref.shape[-1])

    def store_heads(full, ref):
        for h in range(HKV):
            t = full[:, REP * h * DH:(REP * h + 1) * DH]
            for r in range(1, REP):
                t = jnp.where(row % REP == r, full[:, (REP * h + r) * DH:(REP * h + r + 1) * DH], t)
            ref[h] = t

    for c in small_in:
        c.wait()
    x, go = tile(x_ref), tile(go_ref)
    gw = gw_ref[...].astype(F32).reshape(1, D)
    gate = jax.nn.sigmoid(jnp.sum(x * gw, axis=-1, keepdims=True))
    da = (gate * go).astype(BF16)
    db = ((1.0 - gate) * go).astype(BF16)
    xb = x.astype(BF16)

    pltpu.make_async_copy(w1_hbm, w1_ref, sem_1).wait()
    pltpu.make_async_copy(w2_hbm, w2_ref, sem_2).wait()
    pltpu.make_async_copy(wq_hbm, wq_ref, sem_q).wait()
    pltpu.make_async_copy(wo_hbm, wo_ref, sem_o).wait()
    prologue_reads()
    store_heads(_dot(xb, matrix(wq_ref)), q_ref)
    prologue_reads()
    store_heads(_dot(da, matrix(wo_ref), NT), do_ref)
    prologue_reads()

    h_pre = _dot(xb, matrix(w1_ref)).astype(BF16).astype(F32)
    act = jnp.maximum(h_pre, 0.0).astype(BF16)
    mlp = _dot(act, matrix(w2_ref))
    slope = jnp.where(h_pre > 0.0, 1.0, jnp.where(h_pre == 0.0, 0.5, 0.0))
    dh = (_dot(db, matrix(w2_ref), NT) * slope).astype(BF16)
    dx = _dot(dh, matrix(w1_ref), NT)
    prologue_reads()
    once = row % REP == 0
    dw1_ref[...] = _dot(jnp.where(once, x, 0.0).astype(BF16), dh, TN).astype(BF16).reshape(W1_SHAPE)
    prologue_reads()
    dw2_ref[...] = _dot(act, jnp.where(once, db.astype(F32), 0.0).astype(BF16), TN).astype(BF16).reshape(W2_SHAPE)
    read_steps(stage[0], 2 * PART_STEPS + LOOK_AHEAD)
    wait_part(0, part_sems[0])
    wait_part(1, part_sems[1])

    scale = DH ** -0.5

    def pair(p):
        @pl.when(p == SWITCH)
        def _():
            tail = TAIL_ROUNDS * READ_ROWS
            read_last_steps()
            wait_part(2, part_sems[2])
            wait_part(3, part_sems[3], 0, HALF - tail)
            write_caches(0, EARLY_WRITES)
            wait_part(3, sem_tail, HALF - tail, tail)
            write_caches(EARLY_WRITES, _writes_before(SWITCH))

        for i in range(SWITCH + 1, NPAIR):
            pl.when(p == i)(functools.partial(write_caches, _writes_before(i - 1), _writes_before(i)))

        def reads(i):
            @pl.when(p < SWITCH)
            def _():
                lo = 2 * PART_STEPS + LOOK_AHEAD + (4 * p + i) * POINT_STEPS
                read_steps(lo, lo + POINT_STEPS, (2, 3))

        reads(0)
        b, h = p // HKV, p % HKV

        def own_rows(t):
            return jnp.where(low == (b == 0), t, pltpu.roll(t, REP, 0)).astype(BF16)

        q, do = own_rows(q_ref[h]), own_rows(do_ref[h])
        s = jnp.concatenate([_dot(q, k_ref[2 * p + i], NT) for i in range(2)], axis=1) * scale
        dp = jnp.concatenate([_dot(do, v_ref[2 * p + i], NT) for i in range(2)], axis=1)
        e = jnp.exp(s - jnp.max(s, axis=-1, keepdims=True))
        prob = e * (1.0 / jnp.sum(e, axis=-1, keepdims=True))
        ds = prob * (dp - jnp.sum(prob * dp, axis=-1, keepdims=True)) * scale
        both = jnp.where(low, ds, prob)
        both_b = both.astype(BF16)
        reads(1)
        dq_ref[b, h] = sum(_dot(both_b[:, i * HALF:(i + 1) * HALF], k_ref[2 * p + i]) for i in range(2))
        o_ref[b, h] = sum(_dot(both_b[:, i * HALF:(i + 1) * HALF], v_ref[2 * p + i]) for i in range(2))

        blocks = 128 // 8
        rows = SK // blocks
        folded = jnp.concatenate([both[:, j * rows:(j + 1) * rows] for j in range(blocks)], axis=0)
        folded = folded.T.astype(BF16)
        for_k = jnp.tile(jnp.where(low, q.astype(F32), 0.0), (blocks, 1))
        for_v = jnp.tile(jnp.where(low, 0.0, do.astype(F32)), (blocks, 1))
        block = lax.broadcasted_iota(jnp.int32, (128, DH), 0) // 8
        for j in range(blocks):
            if j in (3, 9):
                reads(2 + j // 8)
            i, at = divmod(j * rows, HALF)
            k_ref[2 * p + i, at:at + rows] = _dot(folded, jnp.where(block == j, for_k, 0.0).astype(BF16)).astype(BF16)
            v_ref[2 * p + i, at:at + rows] = _dot(folded, jnp.where(block == j, for_v, 0.0).astype(BF16)).astype(BF16)

    _loop(0, NPAIR, pair)

    def spread_heads(ref, high):
        cols = []
        for h in range(HKV):
            t0, t1 = ref[0, h], ref[1, h]
            if high:
                t = jnp.where(low, pltpu.roll(t0, REP, 0), t1)
            else:
                t = jnp.where(low, t0, pltpu.roll(t1, REP, 0))
            cols += [jnp.where(row % REP == r, t, 0.0) for r in range(REP)]
        return jnp.concatenate(cols, axis=1).astype(BF16)

    def per_token(t):
        return jnp.where(low, jnp.sum(t[:REP], axis=0, keepdims=True), jnp.sum(t[REP:], axis=0, keepdims=True))

    queued = _writes_before(NPAIR - 1)
    write_caches(queued, queued + PAIR_WRITES)
    o = spread_heads(o_ref, True)
    attn = per_token(_dot(o, matrix(wo_ref)))
    dwo_ref[...] = _dot(o, da, TN).astype(BF16).reshape(WO_SHAPE)

    write_caches(queued + PAIR_WRITES, queued + 2 * PAIR_WRITES)
    dq = spread_heads(dq_ref, False)
    dx = dx + per_token(_dot(dq, matrix(wq_ref), NT))
    dwq_ref[...] = _dot(xb, dq, TN).astype(BF16).reshape(WQ_SHAPE)

    dz = jnp.sum(go * (attn - mlp), axis=-1, keepdims=True) * gate * (1.0 - gate)
    out = gate * attn + (1.0 - gate) * mlp
    dx = dx + dz * gw
    dgw = dz * x
    token0 = lax.broadcasted_iota(jnp.int32, (B, 1), 0) == 0
    out_ref[...] = jnp.where(token0, out[0:1], out[REP:REP + 1]).astype(BF16)
    dx_ref[...] = jnp.where(token0, dx[0:1], dx[REP:REP + 1]).astype(BF16)
    dgw_ref[...] = (dgw[0:1] + dgw[REP:REP + 1]).astype(BF16).reshape(D)

    write_caches(queued + 2 * PAIR_WRITES, ALL_WRITES)
    small_out = [pltpu.make_async_copy(src, dst, sem_small)
                 for src, dst in ((out_ref, out_hbm), (dx_ref, dx_hbm), (dgw_ref, dgw_hbm))]
    for c in small_out:
        c.start()
    _loop(0, 64, write_wq_w1)
    _loop(0, 56, functools.partial(write_wo_w2, True))
    _loop(56, 64, functools.partial(write_wo_w2, False))

    for c in small_out:
        c.wait()
    for src, dst, sem in ((k_ref, dk_hbm, sem_k), (v_ref, dv_hbm, sem_v), (dwq_ref, dwq_hbm, sem_q),
                          (dw1_ref, dw1_hbm, sem_1), (dw2_ref, dw2_hbm, sem_2), (dwo_ref, dwo_hbm, sem_o)):
        pltpu.make_async_copy(src, dst, sem).wait()


@jax.jit
def pallas_gated_mix__gqa_block_cached__dense_activation_relu__decode_kernel(
    A_x: jax.Array,
    A_k_cache: jax.Array,
    A_v_cache: jax.Array,
    A_wq: jax.Array,
    A_wo: jax.Array,
    B_x: jax.Array,
    B_w1: jax.Array,
    B_w2: jax.Array,
    gate_w: jax.Array,
    grad_out: jax.Array,
):
    del B_x
    weights = (WQ_SHAPE, WO_SHAPE, W1_SHAPE, W2_SHAPE)
    token, vector = (B, D), (D,)
    hbm = pl.BlockSpec(memory_space=pltpu.HBM)
    out, dx, dk, dv, dwq, dwo, dw1, dw2, dgw = pl.pallas_call(
        _kernel,
        in_specs=[hbm] * 9,
        out_specs=[hbm] * 9,
        out_shape=[jax.ShapeDtypeStruct(s, BF16) for s in (token, token, KV_SHAPE, KV_SHAPE, *weights, vector)],
        scratch_shapes=[
            *(pltpu.VMEM(s, BF16) for s in (KV_SHAPE, KV_SHAPE, *weights, *weights)),
            *(pltpu.VMEM(s, BF16) for s in (token, vector, token, token, token, vector)),
            pltpu.VMEM((HKV, 8, DH), F32), pltpu.VMEM((HKV, 8, DH), F32),
            pltpu.VMEM((B, HKV, 8, DH), F32), pltpu.VMEM((B, HKV, 8, DH), F32),
            pltpu.SemaphoreType.DMA((7,)),
        ],
        compiler_params=pltpu.CompilerParams(vmem_limit_bytes=120 * 1024 * 1024, disable_bounds_checks=True),
    )(A_x.reshape(token), A_k_cache.reshape(KV_SHAPE), A_v_cache.reshape(KV_SHAPE),
      A_wq.reshape(WQ_SHAPE), A_wo.reshape(WO_SHAPE), B_w1.reshape(W1_SHAPE), B_w2.reshape(W2_SHAPE),
      gate_w, grad_out.reshape(token))
    return (out.reshape(A_x.shape), dx.reshape(A_x.shape), dk.reshape(A_k_cache.shape), dv.reshape(A_v_cache.shape),
            dwq.reshape(A_wq.shape), dwo.reshape(A_wo.shape), dw1.reshape(B_w1.shape), dw2.reshape(B_w2.shape), dgw)
```
